```python
import os as _os
_os.environ.setdefault("JAX_PLATFORMS", "cpu")
import jax
import jax.numpy as jnp

def _softmax(x, axis=-1):
    return jax.nn.softmax(x, axis=axis)
def _gelu(x):
    return jax.nn.gelu(x, approximate=True)
def _silu(x):
    return jax.nn.silu(x)
def _sigmoid(x):
    return jax.nn.sigmoid(x)
def _layernorm(x, axis=-1, eps=1e-5):
    m = jnp.mean(x, axis=axis, keepdims=True)
    v = jnp.var(x, axis=axis, keepdims=True)
    return (x - m) / jnp.sqrt(v + eps)
def _scatter_add(tgt, idx, src, axis=0):
    return tgt.at[idx].add(src)
def _segment_sum(src, seg, n):
    return jax.ops.segment_sum(src, seg, n)
class _Rng:
    def __init__(self, key):
        self._k = key
    def _next(self):
        self._k, sub = jax.random.split(self._k)
        return sub
    def normal(self, shape):
        return jax.random.normal(self._next(), shape, dtype=jnp.bfloat16)
    def randint(self, lo, hi, shape):
        return jax.random.randint(self._next(), shape, lo, hi, dtype=jnp.int32)
    def uniform(self, shape, lo=0.0, hi=1.0):
        return jax.random.uniform(self._next(), shape, jnp.bfloat16, lo, hi)
    def permutation(self, n):
        return jax.random.permutation(self._next(), n)


kernel_name = 'interleave_layers__sliding_block_cached__mixer_channel_mlp__decode'

def setup_inputs():
    _rng = _Rng(jax.random.key(int.from_bytes(__import__("os").urandom(4), "little")))
    _w = (lambda a: (lambda t: t.astype(jnp.bfloat16) if jnp.issubdtype(t.dtype, jnp.floating) else t)(jnp.asarray(a)))
    def _A_setup():
        B, Sq, D = 8, 1, 1024
        Hq, Hkv, Sk, Dh = 32, 4, 4096, 128
        assert Hq % Hkv == 0, (Hq, Hkv)
        return {
            "x": _w((lambda *s: _rng.normal(s) * 0.05)(B, Sq, D)),
            "k_cache": _w((lambda *s: _rng.normal(s) * 1.6)(B, Hkv, Sk, Dh)),
            "v_cache": _w((lambda *s: _rng.normal(s) * 0.8)(B, Hkv, Sk, Dh)),
            "wq": _w((lambda *s: _rng.normal(s) * 1.6)(D, Hq * Dh) * (D ** -0.5)),
            "wo": _w((lambda *s: _rng.normal(s) * 0.8)(Hq * Dh, D) * ((Hq * Dh) ** -0.5)),
        }
    _A_in = _A_setup()

    def _B_setup():
        B, S, D, F = 8, 1, 1024, 3584
        return {
            "x": _w((lambda *s: _rng.normal(s) * 0.05)(B, S, D)),
            "w1": _w((lambda *s: _rng.normal(s) * 0.4)(D, F) * (D ** -0.5)),
            "b1": _w((lambda *s: _rng.normal(s) * 0.4)(F)),
            "w2": _w((lambda *s: _rng.normal(s) * 0.4)(F, D) * (F ** -0.5)),
            "b2": _w((lambda *s: _rng.normal(s) * 0.1)(D)),
        }
    _B_in = _B_setup()

    return {
        "A_x": _A_in["x"],
        "A_k_cache": _A_in["k_cache"],
        "A_v_cache": _A_in["v_cache"],
        "A_wq": _A_in["wq"],
        "A_wo": _A_in["wo"],
        "B_x": _B_in["x"],
        "B_w1": _B_in["w1"],
        "B_b1": _B_in["b1"],
        "B_w2": _B_in["w2"],
        "B_b2": _B_in["b2"],
    }

def reference(A_x, A_k_cache, A_v_cache, A_wq, A_wo, B_x, B_w1, B_b1, B_w2, B_b2):
    def _A_ref(x, k_cache, v_cache, wq, wo):
        B, Sq, D = x.shape
        Hq, Dh = 32, 128
        Hkv, Sk = k_cache.shape[1], k_cache.shape[2]
        W = min(4096, max(256, Sk // 4))
        rep = Hq // Hkv
        q = (lambda x, *d: x.transpose(*d))((x @ wq).reshape(B, Sq, Hq, Dh), 0, 2, 1, 3)
        k = jnp.repeat(k_cache[:, :, Sk - W:, :], rep, axis=1)
        v = jnp.repeat(v_cache[:, :, Sk - W:, :], rep, axis=1)
        scores = jnp.einsum("bhqd,bhkd->bhqk", q, k) * (Dh ** -0.5)
        p = _softmax(scores, axis=-1)
        o = jnp.einsum("bhqk,bhkd->bhqd", p, v)
        return (lambda x, *d: x.transpose(*d))(o, 0, 2, 1, 3).reshape(B, Sq, Hq * Dh) @ wo

    def _B_ref(x, w1, b1, w2, b2):
        y = _layernorm(x, axis=-1)
        h = _gelu(jnp.einsum("bsd,df->bsf", y, w1) + b1)
        return jnp.einsum("bsf,fd->bsd", h, w2) + b2

    x = A_x
    x = x + _A_ref(_layernorm(x, axis=-1), A_k_cache, A_v_cache, A_wq, A_wo)
    x = x + _B_ref(_layernorm(x, axis=-1), B_w1, B_b1, B_w2, B_b2)
    x = x + _A_ref(_layernorm(x, axis=-1), A_k_cache, A_v_cache, A_wq, A_wo)
    x = x + _B_ref(_layernorm(x, axis=-1), B_w1, B_b1, B_w2, B_b2)
    return x
```

```python
import jax
import jax.numpy as jnp
from jax import lax
import jax.experimental.pallas as pl
import jax.experimental.pallas.tpu as pltpu

F32 = jnp.float32
BF16 = jnp.bfloat16
I32 = jnp.int32

B, D, HQ, HKV, DH, SK, FF = 8, 1024, 32, 4, 128, 4096, 3584
W = min(4096, max(256, SK // 4))
REP = HQ // HKV
SCALE = DH ** -0.5
EPS = 1e-5
LANES = 128
CHUNK = 512

W2_BLOCKS = (
    (0, 512, 0, 1024),
    (512, 2048, 0, 640), (2048, 3072, 0, 640), (3072, 3584, 0, 640),
    (512, 2560, 640, 896), (2560, 3328, 640, 896), (3328, 3584, 640, 896),
    (512, 1792, 896, 1024), (1792, 3072, 896, 1024), (3072, 3584, 896, 1024),
)


def _dot(a, b):
    return jnp.dot(a, b, preferred_element_type=F32)


def _ln_stats(x):
    mean = jnp.mean(x, axis=-1, keepdims=True)
    c = x - mean
    rstd = lax.rsqrt(jnp.mean(c * c, axis=-1, keepdims=True) + EPS)
    return mean, rstd, c * rstd


def _ln_proj(x, scale):
    mean, rstd, _ = _ln_stats(x)
    mul = rstd * scale
    return lambda t, cs: (t - mean * cs) * mul


def _ln_ln_proj(x):
    mean, rstd, y = _ln_stats(x)
    mean2, rstd2, _ = _ln_stats(y)
    return lambda t, cs: ((t - mean * cs) * rstd - mean2 * cs) * rstd2


def _gelu(x):
    return 0.5 * x * (1.0 + jnp.tanh(0.7978845608028654 * (x + 0.044715 * (x * x * x))))


def _round(x):
    xb = x.astype(BF16)
    return xb, xb.astype(F32)


def _pack(w):
    return pltpu.bitcast(w, I32)


def _unpack(words):
    return pltpu.bitcast(words, BF16)


def _ds(start, size):
    return pl.ds(pl.multiple_of(start, size), size)


def _heads_of(b, g):
    return pl.ds(g * (REP * B) + b, REP, stride=B)


def _bias_tile(bias, j):
    return jnp.broadcast_to(bias[j:j + 1, :], (B, LANES))


def _kernel(x_hbm, k_hbm, v_hbm, wq_hbm, wo_hbm, w1_hbm, b1_hbm, w2_hbm, b2_hbm, o_ref,
            x_v, b1_v, b2_v, wq_r, k_r, v_r, wo_r, w1_r, w2_r,
            wq_p, kt_p, v_p, wo_p, w1_p, w2_p,
            q_s, o_s, ob_s, qa_s, csq_s, cs1_s, b1_s, h_s, p_s, l_s):

    def scores(b, g, kt):
        s = _dot(q_s[_heads_of(b, g), :].astype(BF16), kt)
        p = jnp.exp(s - jnp.max(s, axis=-1, keepdims=True))
        p_s[g * B + b] = p
        l_s[g * B + b] = jnp.broadcast_to(1.0 / jnp.sum(p, axis=-1, keepdims=True), (REP, DH))

    def values(b, g, v):
        o_s[_heads_of(b, g), :] = _dot(p_s[g * B + b].astype(BF16), v) * l_s[g * B + b]

    def layer1(sems):
        copy = pltpu.make_async_copy
        window = pl.ds(SK - W, W)
        c_first = [copy(wq_hbm, wq_r, sems.at[0]), copy(x_hbm, x_v, sems.at[0]),
                   copy(b1_hbm, b1_v, sems.at[0]), copy(b2_hbm, b2_v, sems.at[0])]
        c_k = copy(k_hbm.at[:, :, window, :], k_r, sems.at[1])
        c_v = copy(v_hbm.at[:, :, window, :], v_r, sems.at[2])
        c_wo = copy(wo_hbm, wo_r, sems.at[3])
        c_w1 = copy(w1_hbm, w1_r, sems.at[4])
        c_w2 = [copy(w2_hbm.at[pl.ds(r0, r1 - r0), pl.ds(c0, c1 - c0)],
                     w2_r.at[pl.ds(r0, r1 - r0), pl.ds(c0, c1 - c0)], sems.at[5 + i])
                for i, (r0, r1, c0, c1) in enumerate(W2_BLOCKS)]
        for c in (*c_first, c_k, c_v, c_wo, c_w1, *c_w2):
            c.start()
        for c in c_first:
            c.wait()

        ones = jnp.ones((B, D), BF16)
        x0b = x_v[...]
        x0 = x0b.astype(F32)
        b1 = b1_v[...].astype(F32)
        for j in range(FF // LANES):
            b1_s[:, j * LANES:(j + 1) * LANES] = _bias_tile(b1, j)
        b2 = b2_v[...].astype(F32)
        b2 = jnp.concatenate([_bias_tile(b2, j) for j in range(D // LANES)], axis=1)

        norm = _ln_proj(x0, SCALE)
        lhs = jnp.concatenate([x0b, ones], axis=0)

        @pl.loop(0, HQ * DH // CHUNK)
        def _(c):
            cols = _ds(c * CHUNK, CHUNK)
            w = wq_r[:, cols]
            wq_p[:, cols] = _pack(w)
            t = _dot(lhs, w)
            csq_s[:, cols] = t[B:]
            q = norm(t[:B], t[B:])
            for j in range(CHUNK // DH):
                q_s[_ds((c * (CHUNK // DH) + j) * B, B), :] = q[:, j * DH:(j + 1) * DH]

        c_k.wait()

        @pl.loop(0, B)
        def _(b):
            for g in range(HKV):
                kt = k_r[b, g].T
                kt_p[b, g] = _pack(kt)
                scores(b, g, kt)

        c_v.wait()

        @pl.loop(0, B)
        def _(b):
            for g in range(HKV):
                v = v_r[b, g]
                v_p[b, g] = _pack(v)
                values(b, g, v)

        for h in range(HQ):
            ob_s[:, h * DH:(h + 1) * DH] = o_s[h * B:(h + 1) * B, :]

        c_wo.wait()

        def wo_chunk(c, acc):
            w = wo_r[_ds(c * CHUNK, CHUNK), :]
            wo_p[_ds(c * (CHUNK // 2), CHUNK // 2), :] = _pack(w)
            return acc + _dot(ob_s[:, _ds(c * CHUNK, CHUNK)].astype(BF16), w)

        x1b, x1 = _round(lax.fori_loop(0, HQ * DH // CHUNK, wo_chunk, x0))

        norm1 = _ln_ln_proj(x1)
        lhs1 = jnp.concatenate([x1b, ones], axis=0)
        c_w1.wait()

        @pl.loop(0, FF // CHUNK)
        def _(c):
            cols = _ds(c * CHUNK, CHUNK)
            w = w1_r[:, cols]
            w1_p[:, cols] = _pack(w)
            t = _dot(lhs1, w)
            cs1_s[:, cols] = t[B:]
            h_s[:, cols] = _gelu(norm1(t[:B], t[B:]) + b1_s[:, cols])

        base = x1 + b2
        tiles = [base[:, j * LANES:(j + 1) * LANES] for j in range(D // LANES)]
        x2b = None
        for c, (r0, r1, c0, c1) in zip(c_w2, W2_BLOCKS):
            c.wait()
            w = w2_r[r0:r1, c0:c1]
            w2_p[r0 // 2:r1 // 2, c0:c1] = _pack(w)
            acc = jnp.concatenate(tiles[c0 // LANES:c1 // LANES], axis=1)
            acc = acc + _dot(h_s[:, r0:r1].astype(BF16), w)
            if r1 == FF:
                x2b, acc = _round(acc)
                if c1 < D:
                    t = _dot(x2b, _unpack(wq_p[c0 // 2:c1 // 2, :]))
                    qa_s[...] = t if c0 == 0 else qa_s[...] + t
            for j in range((c1 - c0) // LANES):
                tiles[c0 // LANES + j] = acc[:, j * LANES:(j + 1) * LANES]
        return jnp.concatenate(tiles, axis=1), x2b, b2

    x2, x2b_last, b2 = pl.run_scoped(
        layer1, pltpu.SemaphoreType.DMA((5 + len(W2_BLOCKS),)))

    norm = _ln_proj(x2, SCALE)
    last = W2_BLOCKS[-1][2]
    for g in range(HKV):
        cols = slice(g * REP * DH, (g + 1) * REP * DH)
        t = qa_s[:, cols] + _dot(x2b_last, _unpack(wq_p[last // 2:, cols]))
        q = norm(t, csq_s[:, cols])
        for j in range(REP):
            q_s[(g * REP + j) * B:(g * REP + j + 1) * B, :] = q[:, j * DH:(j + 1) * DH]
    for g in range(HKV):
        for b in range(B):
            scores(b, g, _unpack(kt_p[b, g]))
    for g in range(HKV):
        for b in range(B):
            values(b, g, _unpack(v_p[b, g]))

    half = D // 2
    rows = REP * DH // 2
    halves = []
    for c in range(2):
        cols = slice(c * half, (c + 1) * half)
        acc = x2[:, cols]
        for g in range(HKV):
            o = jnp.concatenate(
                [o_s[(g * REP + j) * B:(g * REP + j + 1) * B, :] for j in range(REP)], axis=1)
            acc = acc + _dot(o.astype(BF16), _unpack(wo_p[g * rows:(g + 1) * rows, cols]))
        halves.append(_round(acc))
    x3b = jnp.concatenate([halves[0][0], halves[1][0]], axis=1)
    x3 = jnp.concatenate([halves[0][1], halves[1][1]], axis=1)

    norm = _ln_ln_proj(x3)
    head = 1024
    h_s[:, :head] = _dot(halves[0][0], _unpack(w1_p[:half // 2, :head]))
    t = jnp.concatenate([
        h_s[:, :head] + _dot(halves[1][0], _unpack(w1_p[half // 2:, :head])),
        _dot(x3b, _unpack(w1_p[:, head:])),
    ], axis=1)
    h = _gelu(norm(t, cs1_s[...]) + b1_s[...]).astype(BF16)
    o_ref[...] = (x3 + b2 + _dot(h, _unpack(w2_p[...]))).astype(o_ref.dtype)


@jax.jit
def pallas_interleave_layers__sliding_block_cached__mixer_channel_mlp__decode_kernel(A_x, A_k_cache, A_v_cache, A_wq, A_wo, B_x, B_w1, B_b1, B_w2, B_b2):
    del B_x
    assert A_x.shape == (B, 1, D) and A_k_cache.shape == A_v_cache.shape == (B, HKV, SK, DH)
    assert A_wq.shape == (D, HQ * DH) and B_w1.shape == (D, FF)
    vmem = pltpu.VMEM
    out = pl.pallas_call(
        _kernel,
        out_shape=jax.ShapeDtypeStruct((B, D), A_x.dtype),
        in_specs=[pl.BlockSpec(memory_space=pltpu.MemorySpace.HBM)] * 9,
        scratch_shapes=[
            vmem((B, D), BF16), vmem((FF // LANES, LANES), BF16), vmem((D // LANES, LANES), BF16),
            vmem((D, HQ * DH), BF16), vmem((B, HKV, W, DH), BF16), vmem((B, HKV, W, DH), BF16),
            vmem((HQ * DH, D), BF16), vmem((D, FF), BF16), vmem((FF, D), BF16),
            vmem((D // 2, HQ * DH), I32), vmem((B, HKV, DH // 2, W), I32),
            vmem((B, HKV, W // 2, DH), I32), vmem((HQ * DH // 2, D), I32),
            vmem((D // 2, FF), I32), vmem((FF // 2, D), I32),
            vmem((HQ * B, DH), F32), vmem((HQ * B, DH), F32),
            vmem((B, HQ * DH), F32), vmem((B, HQ * DH), F32), vmem((B, HQ * DH), F32),
            vmem((B, FF), F32), vmem((B, FF), F32), vmem((B, FF), F32),
            vmem((HKV * B, REP, W), F32), vmem((HKV * B, REP, DH), F32),
        ],
        compiler_params=pltpu.CompilerParams(vmem_limit_bytes=110 * 1024 * 1024),
        name="fused_decode",
    )(A_x.reshape(B, D), A_k_cache, A_v_cache, A_wq, A_wo, B_w1,
      B_b1.reshape(FF // LANES, LANES), B_w2, B_b2.reshape(D // LANES, LANES))
    return out.reshape(B, 1, D)
```
